```python
import os as _os
_os.environ.setdefault("JAX_PLATFORMS", "cpu")
import jax
import jax.numpy as jnp

def _softmax(x, axis=-1):
    return jax.nn.softmax(x, axis=axis)
def _gelu(x):
    return jax.nn.gelu(x, approximate=True)
def _silu(x):
    return jax.nn.silu(x)
def _sigmoid(x):
    return jax.nn.sigmoid(x)
def _layernorm(x, axis=-1, eps=1e-5):
    m = jnp.mean(x, axis=axis, keepdims=True)
    v = jnp.var(x, axis=axis, keepdims=True)
    return (x - m) / jnp.sqrt(v + eps)
def _scatter_add(tgt, idx, src, axis=0):
    return tgt.at[idx].add(src)
def _segment_sum(src, seg, n):
    return jax.ops.segment_sum(src, seg, n)
class _Rng:
    def __init__(self, key):
        self._k = key
    def _next(self):
        self._k, sub = jax.random.split(self._k)
        return sub
    def normal(self, shape):
        return jax.random.normal(self._next(), shape, dtype=jnp.bfloat16)
    def randint(self, lo, hi, shape):
        return jax.random.randint(self._next(), shape, lo, hi, dtype=jnp.int32)
    def uniform(self, shape, lo=0.0, hi=1.0):
        return jax.random.uniform(self._next(), shape, jnp.bfloat16, lo, hi)
    def permutation(self, n):
        return jax.random.permutation(self._next(), n)


kernel_name = 'interleave_layers__linear_attn_block__mha_block__prompt'

def setup_inputs():
    _rng = _Rng(jax.random.key(int.from_bytes(__import__("os").urandom(4), "little")))
    _w = (lambda a: (lambda t: t.astype(jnp.bfloat16) if jnp.issubdtype(t.dtype, jnp.floating) else t)(jnp.asarray(a)))
    def _A_setup():
        B, S, D = 1, 2048, 640
        return {
            "x": _w((lambda *s: _rng.normal(s) * 0.05)(B, S, D)),
            "wqkv": _w((lambda *s: _rng.normal(s) * 0.1)(D, 3 * D)),
            "wo": _w((lambda *s: _rng.normal(s) * 0.05)(D, D)),
        }
    _A_in = _A_setup()

    def _B_setup():
        B, S, D, H = 1, 2048, 640, 32
        return {
            "x": _w((lambda *s: _rng.normal(s) * 0.05)(B, S, D)),
            "wqkv": _w((lambda *s: _rng.normal(s) * 0.1)(D, 3 * D)),
            "wo": _w((lambda *s: _rng.normal(s) * 0.05)(D, D)),
        }
    _B_in = _B_setup()

    return {
        "A_x": _A_in["x"],
        "A_wqkv": _A_in["wqkv"],
        "A_wo": _A_in["wo"],
        "B_x": _B_in["x"],
        "B_wqkv": _B_in["wqkv"],
        "B_wo": _B_in["wo"],
    }

def reference(A_x, A_wqkv, A_wo, B_x, B_wqkv, B_wo):
    def _A_ref(x, wqkv, wo):
        B, S, D = x.shape
        H = 32; Dh = D // H
        qkv = (lambda x, *d: x.transpose(*d))((x @ wqkv).reshape(B, S, 3, H, Dh), 2, 0, 3, 1, 4)
        q, k, v = qkv[0], qkv[1], qkv[2]
        phi = lambda t: jnp.where(t > 0, t + 1, jnp.exp(t)) + 1e-6
        pq, pk = phi(q), phi(k)
        kv = jnp.einsum("bhsd,bhse->bhde", pk, v)
        z = jnp.einsum("bhsd->bhd", pk)
        num = jnp.einsum("bhqd,bhde->bhqe", pq, kv)
        den = jnp.einsum("bhqd,bhd->bhq", pq, z)[..., None] + 1e-6
        o = num / den
        return (lambda x, *d: x.transpose(*d))(o, 0, 2, 1, 3).reshape(B, S, D) @ wo

    def _B_ref(x, wqkv, wo):
        B, S, D = x.shape
        H = 32
        Dh = D // H
        qkv = (lambda x, *d: x.transpose(*d))((x @ wqkv).reshape(B, S, 3, H, Dh), 2, 0, 3, 1, 4)
        q, k, v = qkv[0], qkv[1], qkv[2]
        scores = jnp.einsum("bhqd,bhkd->bhqk", q, k) * (Dh ** -0.5)
        p = _softmax(scores, axis=-1)
        o = jnp.einsum("bhqk,bhkd->bhqd", p, v)
        return (lambda x, *d: x.transpose(*d))(o, 0, 2, 1, 3).reshape(B, S, D) @ wo

    x = A_x
    x = x + _A_ref(_layernorm(x, axis=-1), A_wqkv, A_wo)
    x = x + _B_ref(_layernorm(x, axis=-1), B_wqkv, B_wo)
    x = x + _A_ref(_layernorm(x, axis=-1), A_wqkv, A_wo)
    x = x + _B_ref(_layernorm(x, axis=-1), B_wqkv, B_wo)
    return x
```

```python
import jax
import jax.numpy as jnp
from jax import lax
import jax.experimental.pallas as pl
import jax.experimental.pallas.tpu as pltpu

S, D, H, DH = 2048, 640, 32, 20
TC = 512
BQ = 512
NS = S // BQ
BK = 128
NC = S // BK
LEAD = 3
NSLAB = 6
F32, BF16 = jnp.float32, jnp.bfloat16
LOG2E = 1.4426950408889634
NT = (((1,), (1,)), ((), ()))
TN = (((0,), (0,)), ((), ()))

BANDS = []
for _j in range(D // 128):
    _h0 = (128 * _j) // DH
    _h1 = -(-(128 * (_j + 1)) // DH)
    BANDS.append(((_h0 * DH) // 8 * 8, min(D, -(-(_h1 * DH) // 8) * 8)))


def _slab_start(s):
    return min(120 * s, D - 128)


def _layernorm(x):
    m = jnp.mean(x, axis=-1, keepdims=True)
    xc = x - m
    v = jnp.mean(xc * xc, axis=-1, keepdims=True)
    return xc * lax.rsqrt(v + 1e-5)


def _phi(t):
    return jnp.where(t > 0, t + 1.0, jnp.exp(t)) + 1e-6


def _rnd(t):
    return t.astype(BF16).astype(F32)


def _kernel(x_hbm, awqkv_hbm, awo_hbm, bwqkv_hbm, bwo_hbm, out_hbm,
            xin, awqkv, awo, bwqkv, bwo, awqvt, bwqvt, bwk, xres,
            qt, ks, vt, ot, sbuf, mbuf, kvt, zsum, mmat, zsel, sems):
    cp_x = pltpu.make_async_copy(x_hbm, xin, sems.at[0])
    cp_aw = pltpu.make_async_copy(awqkv_hbm, awqkv, sems.at[1])
    cp_ao = pltpu.make_async_copy(awo_hbm, awo, sems.at[2])
    cp_bw = pltpu.make_async_copy(bwqkv_hbm, bwqkv, sems.at[3])
    cp_bo = pltpu.make_async_copy(bwo_hbm, bwo, sems.at[4])
    cp_aw.start()
    cp_x.start()
    cp_bw.start()
    cp_ao.start()
    cp_bo.start()

    def prep_t(w, wt):
        for part, c0 in ((0, 0), (1, 2 * D)):
            for j in range(D // 128):
                blk = w[:, c0 + 128 * j:c0 + 128 * (j + 1)]
                wt[part * D + 128 * j:part * D + 128 * (j + 1), :] = blk.T

    cp_aw.wait()
    prep_t(awqkv, awqvt)
    cp_x.wait()

    def cast_in(i, c):
        r = pl.ds(pl.multiple_of(i * TC, TC), TC)
        xres[r, :] = xin[r, :].astype(F32)
        return c
    lax.fori_loop(0, S // TC, cast_in, 0)

    cp_bw.wait()
    prep_t(bwqkv, bwqvt)
    for s in range(NSLAB):
        c0 = D + _slab_start(s)
        bwk[:, 128 * s:128 * (s + 1)] = bwqkv[:, c0:c0 + 128]
    cp_ao.wait()
    cp_bo.wait()

    def layer_a():
        kvt[...] = jnp.zeros(kvt.shape, F32)
        zsum[...] = jnp.zeros(zsum.shape, F32)

        def pass1(i, c):
            t0 = pl.multiple_of(i * TC, TC)
            xn = _layernorm(xres[pl.ds(t0, TC), :]).astype(BF16)
            k = jnp.dot(xn, awqkv[:, D:2 * D], preferred_element_type=F32)
            pk = _phi(k)
            zsum[...] += jnp.sum(pk.reshape(TC // 8, 8, D), axis=0)
            pkb = pk.astype(BF16)
            qv = lax.dot_general(awqvt[...], xn, NT, preferred_element_type=F32)
            qt[:, pl.ds(t0, TC)] = _phi(qv[:D])
            v = _rnd(qv[D:])
            for j, (r0, r1) in enumerate(BANDS):
                kvt[r0:r1, 128 * j:128 * (j + 1)] += jnp.dot(
                    v[r0:r1], pkb[:, 128 * j:128 * (j + 1)], preferred_element_type=F32)
            return c
        lax.fori_loop(0, S // TC, pass1, 0)

        re = lax.broadcasted_iota(jnp.int32, (D, D), 0) // DH
        cd = lax.broadcasted_iota(jnp.int32, (D, D), 1) // DH
        kvb = jnp.where(re == cd, kvt[...], 0.0).astype(BF16)
        mmat[...] = lax.dot_general(kvb, awo[...], TN, preferred_element_type=F32).astype(BF16)
        z = jnp.sum(zsum[...], axis=0, keepdims=True)
        rh = lax.broadcasted_iota(jnp.int32, (H, D), 0)
        ch = lax.broadcasted_iota(jnp.int32, (H, D), 1) // DH
        zsel[...] = jnp.where(rh == ch, z, 0.0).astype(BF16)

        def pass2(i, c):
            t0 = pl.multiple_of(i * TC, TC)
            pq = qt[:, pl.ds(t0, TC)]
            den = jnp.dot(zsel[...], pq.astype(BF16), preferred_element_type=F32) + 1e-6
            rden = 1.0 / den
            row = lax.broadcasted_iota(jnp.int32, (8, TC), 0)
            parts = []
            for j in range(H // 2):
                r0 = jnp.broadcast_to(rden[2 * j:2 * j + 1], (8, TC))
                r1 = jnp.broadcast_to(rden[2 * j + 1:2 * j + 2], (8, TC))
                parts += [r0, r0, jnp.where(row < 4, r0, r1), r1, r1]
            pn = (pq * jnp.concatenate(parts, axis=0)).astype(BF16)
            o = lax.dot_general(pn, mmat[...], TN, preferred_element_type=F32)
            xres[pl.ds(t0, TC), :] += o
            return c
        lax.fori_loop(0, S // TC, pass2, 0)

    def substep(h_cur, j_cur, h_nxt, j_nxt):
        do_pv, do_qk = h_cur is not None, h_nxt is not None
        if do_qk:
            sl = (h_nxt * 43) >> 8
            st = jnp.minimum(sl * 120, D - 128)
            off = h_nxt * DH - st
            q = qt[pl.ds(pl.multiple_of(st, 8), 128), j_nxt * BQ:(j_nxt + 1) * BQ]
            r = lax.broadcasted_iota(jnp.int32, (128, BQ), 0)
            q = jnp.where((r >= off) & (r < off + DH), q, 0.0).astype(BF16)
            m_n = jnp.full((8, BQ), -jnp.inf, F32)
        if do_pv:
            m_cur = mbuf[:, j_cur * BQ:(j_cur + 1) * BQ]
            acc = jnp.zeros((24, BQ), F32)
        for c in range(NC):
            ck = slice(c * BK, (c + 1) * BK)
            if do_qk:
                s = jnp.dot(ks[sl, ck, :], q, preferred_element_type=F32)
                sbuf[j_nxt, ck, :] = s
                m_n = jnp.maximum(m_n, jnp.max(s.reshape(BK // 8, 8, BQ), axis=0))
            if do_pv:
                p = jnp.exp2(sbuf[j_cur, ck, :] - m_cur).astype(BF16)
                acc = acc + jnp.dot(vt[h_cur, :, ck], p, preferred_element_type=F32)
        if do_qk:
            mbuf[:, j_nxt * BQ:(j_nxt + 1) * BQ] = jnp.max(m_n, axis=0, keepdims=True)
        if do_pv:
            lo = (h_cur & 1) * 4
            l = jnp.where(lo > 0, acc[0:1], acc[20:21])
            o = acc * (1.0 / l)
            r = lax.broadcasted_iota(jnp.int32, (24, BQ), 0)
            rows = pl.ds(pl.multiple_of(h_cur * DH - lo, 8), 24)
            cols = slice(j_cur * BQ, (j_cur + 1) * BQ)
            ot[rows, cols] = jnp.where((r >= lo) & (r < lo + DH), o, ot[rows, cols])

    def layer_b(last):
        def proj(i, c):
            t0 = pl.multiple_of(i * TC, TC)
            tok = pl.ds(t0, TC)
            xn = _layernorm(xres[tok, :]).astype(BF16)
            k = jnp.dot(xn, bwk[...], preferred_element_type=F32).astype(BF16)
            for s in range(NSLAB):
                ks[s, tok, :] = k[:, 128 * s:128 * (s + 1)]
            qv = lax.dot_general(bwqvt[...], xn, NT, preferred_element_type=F32)
            qt[:, tok] = qv[:D] * (LOG2E * DH ** -0.5)
            v = _rnd(qv[D:])
            row = lax.broadcasted_iota(jnp.int32, (8, TC), 0)
            for j in range(H // 2):
                b = 40 * j
                mid = v[b + 16:b + 24]
                vt[2 * j, 0:16, tok] = v[b:b + 16]
                vt[2 * j, 16:24, tok] = jnp.where(row < 4, mid, 1.0)
                vt[2 * j + 1, 0:8, tok] = jnp.where(row < 4, 1.0, mid)
                vt[2 * j + 1, 8:24, tok] = v[b + 24:b + 40]
            return c
        lax.fori_loop(0, S // TC, proj, 0)

        for j in range(LEAD):
            substep(None, None, 0, j)

        def head(h, c):
            for j in range(NS):
                jn = j + LEAD
                substep(h, j, h + jn // NS, jn % NS)
            return c
        lax.fori_loop(0, H - 1, head, 0)
        for j in range(NS):
            jn = j + LEAD
            substep(H - 1, j, H - 1 if jn < NS else None, jn if jn < NS else None)

        def out_copy(i):
            tok = pl.ds(pl.multiple_of(i * TC, TC), TC)
            return pltpu.make_async_copy(xin.at[tok, :], out_hbm.at[tok, :], sems.at[i])

        def oproj(i, c):
            tok = pl.ds(pl.multiple_of(i * TC, TC), TC)
            o = lax.dot_general(ot[:, tok].astype(BF16), bwo[...], TN, preferred_element_type=F32)
            xnew = xres[tok, :] + o
            xres[tok, :] = xnew
            xin[tok, :] = xnew.astype(BF16)

            @pl.when(last)
            def _():
                out_copy(i).start()
            return c
        lax.fori_loop(0, S // TC, oproj, 0)

        @pl.when(last)
        def _():
            for i in range(S // TC):
                out_copy(i).wait()

    ot[...] = jnp.zeros(ot.shape, F32)

    def rep(r, c):
        layer_a()
        layer_b(r == 1)
        return c
    lax.fori_loop(0, 2, rep, 0)


@jax.jit
def pallas_interleave_layers__linear_attn_block__mha_block__prompt_kernel(
    A_x: jax.Array,
    A_wqkv: jax.Array,
    A_wo: jax.Array,
    B_x: jax.Array,
    B_wqkv: jax.Array,
    B_wo: jax.Array,
):
    del B_x
    any_spec = pl.BlockSpec(memory_space=pl.ANY)
    out = pl.pallas_call(
        _kernel,
        out_shape=jax.ShapeDtypeStruct((S, D), BF16),
        in_specs=[any_spec] * 5,
        out_specs=any_spec,
        scratch_shapes=[
            pltpu.VMEM((S, D), BF16),
            pltpu.VMEM((D, 3 * D), BF16),
            pltpu.VMEM((D, D), BF16),
            pltpu.VMEM((D, 3 * D), BF16),
            pltpu.VMEM((D, D), BF16),
            pltpu.VMEM((2 * D, D), BF16),
            pltpu.VMEM((2 * D, D), BF16),
            pltpu.VMEM((D, NSLAB * 128), BF16),
            pltpu.VMEM((S, D), F32),
            pltpu.VMEM((D, S), F32),
            pltpu.VMEM((NSLAB, S, 128), BF16),
            pltpu.VMEM((H, 24, S), F32),
            pltpu.VMEM((D, S), F32),
            pltpu.VMEM((NS, S, BQ), F32),
            pltpu.VMEM((1, S), F32),
            pltpu.VMEM((D, D), F32),
            pltpu.VMEM((8, D), F32),
            pltpu.VMEM((D, D), BF16),
            pltpu.VMEM((H, D), BF16),
            pltpu.SemaphoreType.DMA((5,)),
        ],
        compiler_params=pltpu.CompilerParams(vmem_limit_bytes=110 * 1024 * 1024),
        name="interleave_layers",
    )(A_x.reshape(S, D), A_wqkv, A_wo, B_wqkv, B_wo)
    return out.reshape(1, S, D)
```

```python
import jax
import jax.numpy as jnp
from jax import lax
import jax.experimental.pallas as pl
import jax.experimental.pallas.tpu as pltpu

S, D, H, DH = 2048, 640, 32, 20
TC = 512
NQ = S // TC
BK = 128
NC = S // BK
LEAD = 2
RING = LEAD + 1
BODY = 9
NSTEP = H * NQ
assert (NSTEP - LEAD) % BODY == 0 and BODY % RING == 0
NSLAB = 6
NTILE = D // 128
NP = 8
F32, BF16 = jnp.float32, jnp.bfloat16
LOG2E = 1.4426950408889634
NN = (((1,), (0,)), ((), ()))
NT = (((1,), (1,)), ((), ()))
TN = (((0,), (0,)), ((), ()))


def _bands(align):
    out = []
    for j in range(NTILE):
        h0 = (128 * j) // DH
        h1 = -(-(128 * (j + 1)) // DH)
        out.append(((h0 * DH) // align * align, min(D, -(-(h1 * DH) // align) * align)))
    return out


def _layernorm(x):
    m = jnp.mean(x, axis=-1, keepdims=True)
    xc = x - m
    v = jnp.mean(xc * xc, axis=-1, keepdims=True)
    return xc * lax.rsqrt(v + 1e-5)


def _phi(t):
    return jnp.where(t > 0, t + 1.0, jnp.exp(t)) + 1e-6


def _rnd(t):
    return t.astype(BF16).astype(F32)


def _recip(l):
    r = pltpu.reciprocal(l, approx=True)
    return r * (2.0 - l * r)


def _head_of(i):
    return (i * 3277) >> 16


def _pace(never, a, side, p, first):
    rows = a.shape[0]
    for t in range(NP):
        if first + t * (NP - first) // NP == p:
            a = jnp.where(never, side[t * rows:(t + 1) * rows], a)
    return a


def _paced_dot(never, lhs, rhs, side, dims=NN, first=2):
    rows = lhs.shape[0] // NP
    return [lax.dot_general(_pace(never, lhs[p * rows:(p + 1) * rows], side, p, first), rhs[...],
                            dims, preferred_element_type=F32) for p in range(NP)]


def _chunk(i):
    if isinstance(i, int):
        return pl.ds(i * TC, TC)
    return pl.ds(pl.multiple_of(i * TC, TC), TC)


def _loop(n, body):
    def wrapped(i, c):
        body(i)
        return c
    lax.fori_loop(0, n, wrapped, 0)


def _kernel(x_hbm, awqkv_hbm, awo_hbm, bwqkv_hbm, bwo_hbm, out_hbm,
            xio, awqkv, awo, bwqkv, bwo, awqvt, bwqvt, xres, xn, xn1, pkb,
            qt, ks, vt, ot, lhs, qs, sbuf, mbuf, kvt, zsum, mmat, zsel, sems):
    def col_copy(part, sem):
        cols = slice(part * D, (part + 1) * D)
        return pltpu.make_async_copy(awqkv_hbm.at[:, cols], awqkv.at[:, cols], sems.at[sem])

    def in_copy(i):
        return pltpu.make_async_copy(x_hbm.at[_chunk(i), :], xio.at[_chunk(i), :], sems.at[i])

    def out_copy(i):
        return pltpu.make_async_copy(xio.at[_chunk(i), :], out_hbm.at[_chunk(i), :], sems.at[i])

    cp_wq, cp_wk, cp_wv = col_copy(0, 4), col_copy(1, 5), col_copy(2, 6)
    cp_ao = pltpu.make_async_copy(awo_hbm, awo, sems.at[7])
    cp_bw = pltpu.make_async_copy(bwqkv_hbm, bwqkv, sems.at[8])
    cp_bo = pltpu.make_async_copy(bwo_hbm, bwo, sems.at[9])

    def transpose_qv(w, wt):
        for part, c0 in ((0, 0), (1, 2 * D)):
            for j in range(NTILE):
                blk = w[:, c0 + 128 * j:c0 + 128 * (j + 1)]
                wt[part * D + 128 * j:part * D + 128 * (j + 1), :] = blk.T

    def norm(i):
        return _layernorm(xres[_chunk(i), :]).astype(BF16)

    def nxt(i):
        return jnp.minimum(i + 1, NQ - 1)

    def lin_k(i):
        y = norm(nxt(i))
        x = xn1[...]
        xn[_chunk(i), :] = x
        pk = _phi(jnp.concatenate(_paced_dot(i < 0, x, awqkv.at[:, D:2 * D], y), axis=0))
        zsum[...] += jnp.sum(pk.reshape(TC // 8, 8, D), axis=0)
        pkb[_chunk(i), :] = pk.astype(BF16)
        xn1[...] = y

    def lin_qv(i):
        tok = _chunk(i)
        x = xn[tok, :]
        v = _rnd(lax.dot_general(awqvt[D:, :], x, NT, preferred_element_type=F32))
        for j, (r0, r1) in enumerate(_bands(8)):
            kvt[r0:r1, 128 * j:128 * (j + 1)] += jnp.dot(
                v[r0:r1], pkb[tok, 128 * j:128 * (j + 1)], preferred_element_type=F32)
        qt[:, tok] = _phi(lax.dot_general(awqvt[:D, :], x, NT, preferred_element_type=F32))

    def fold_kv():
        z = jnp.sum(zsum[...], axis=0, keepdims=True)
        rh = lax.broadcasted_iota(jnp.int32, (H, D), 0)
        ch = _head_of(lax.broadcasted_iota(jnp.int32, (H, D), 1))
        zsel[...] = jnp.where(rh == ch, z, 0.0).astype(BF16)
        for j, (r0, r1) in enumerate(_bands(16)):
            re = _head_of(lax.broadcasted_iota(jnp.int32, (r1 - r0, 128), 0) + r0)
            cd = _head_of(lax.broadcasted_iota(jnp.int32, (r1 - r0, 128), 1) + 128 * j)
            kvb = jnp.where(re == cd, kvt[r0:r1, 128 * j:128 * (j + 1)], 0.0).astype(BF16)
            mmat[128 * j:128 * (j + 1), :] = lax.dot_general(
                kvb, awo[r0:r1, :], TN, preferred_element_type=F32).astype(BF16)

    def scaled_q(i):
        pq = qt[:, _chunk(i)]
        den = jnp.dot(zsel[...], pq.astype(BF16), preferred_element_type=F32) + 1e-6
        rden = 1.0 / den
        row = lax.broadcasted_iota(jnp.int32, (8, TC), 0)
        parts = []
        for j in range(H // 2):
            r0 = jnp.broadcast_to(rden[2 * j:2 * j + 1], (8, TC))
            r1 = jnp.broadcast_to(rden[2 * j + 1:2 * j + 2], (8, TC))
            parts += [r0, r0, jnp.where(row < 4, r0, r1), r1, r1]
        return (pq * jnp.concatenate(parts, axis=0)).astype(BF16).T

    def lin_out(i, never, final=False):
        side = norm(0) if final else scaled_q(i + 1)
        xres[_chunk(i), :] += jnp.concatenate(_paced_dot(never, lhs[...], mmat, side), axis=0)
        (xn1 if final else lhs)[...] = side

    def mha_qkv(i):
        tok = _chunk(i)
        y = norm(nxt(i))
        x = xn1[...]
        k = jnp.dot(x, bwqkv[:, D:2 * D], preferred_element_type=F32)
        lane = lax.broadcasted_iota(jnp.int32, (TC, 128), 1)
        ks[0, tok, :] = k[:, :128].astype(BF16)
        ks[NSLAB - 1, tok, :] = k[:, D - 128:].astype(BF16)
        for s in range(1, NSLAB - 1):
            mix = jnp.where(lane >= 128 - 8 * s, k[:, 128 * (s - 1):128 * s], k[:, 128 * s:128 * (s + 1)])
            ks[s, tok, :] = pltpu.roll(mix, 8 * s, 1).astype(BF16)
        v = _rnd(lax.dot_general(bwqvt[D:, :], x, NT, preferred_element_type=F32))
        row = lax.broadcasted_iota(jnp.int32, (8, TC), 0)
        for j in range(H // 2):
            b = 40 * j
            vt[2 * j, 0:16, tok] = v[b:b + 16]
            vt[2 * j, 16:24, tok] = jnp.where(row < 4, v[b + 16:b + 24], 1.0)
            w = [pltpu.roll(v[b + 16 + 8 * t:b + 24 + 8 * t], 4, 0) for t in range(3)] + [1.0]
            for t in range(3):
                vt[2 * j + 1, 8 * t:8 * t + 8, tok] = jnp.where(row < 4, w[t], w[t + 1])
        q = jnp.concatenate(
            [lax.dot_general(bwqvt[:D - TC, :], x, NT, preferred_element_type=F32)]
            + _paced_dot(i < 0, bwqvt[D - TC:D, :], x, y, NT, 0), axis=0)
        q = q * (LOG2E * DH ** -0.5)
        for s in range(NSLAB):
            st = min(120 * s, D - 128)
            qs[s, :, tok] = pltpu.bitcast(q[st:st + 128].astype(BF16), jnp.int32)
        xn1[...] = y

    def step(n_pv, b_pv, n_qk, b_qk, between=None):
        do_pv, do_qk = n_pv is not None, n_qk is not None
        if do_qk:
            h = n_qk >> 2
            sl = (h * 43) >> 8
            off = h * DH - jnp.minimum(sl * 120, D - 128)
            r = lax.broadcasted_iota(jnp.int32, (64, TC), 0) * 2
            q = jnp.where((r >= off) & (r < off + DH), qs[sl, :, _chunk(n_qk & 3)], 0)
            q = pltpu.bitcast(q, BF16)
            m_new = jnp.full((8, TC), -jnp.inf, F32)
        if do_pv:
            hv = n_pv >> 2
            m = jnp.max(mbuf[b_pv], axis=0, keepdims=True)
            acc = jnp.zeros((24, TC), F32)
        for c in range(NC):
            ck = slice(c * BK, (c + 1) * BK)
            if between is not None:
                between(c)
            if do_qk:
                s = jnp.dot(ks[sl, ck, :], q, preferred_element_type=F32)
                sbuf[b_qk, ck, :] = s
                m_new = jnp.maximum(m_new, jnp.max(s.reshape(BK // 8, 8, TC), axis=0))
            if do_pv:
                p = jnp.exp2(sbuf[b_pv, ck, :] - m).astype(BF16)
                acc = acc + jnp.dot(vt[hv, :, ck], p, preferred_element_type=F32)
        if do_qk:
            mbuf[b_qk] = m_new
        if do_pv:
            ot[hv, :, _chunk(n_pv & 3)] = acc

    def gather_o(j):
        tok = _chunk(j)
        row = lax.broadcasted_iota(jnp.int32, (8, TC), 0)
        parts = []
        for p in range(H // 2):
            e, o = ot[2 * p, :, tok], ot[2 * p + 1, :, tok]
            e, o = e * _recip(e[DH:DH + 1]), o * _recip(o[DH:DH + 1])
            w = [e[16:24]] + [pltpu.roll(o[8 * t:8 * t + 8], 4, 0) for t in range(3)]
            parts += [e[0:16]] + [jnp.where(row < 4, w[t], w[t + 1]) for t in range(3)]
        return jnp.concatenate(parts, axis=0).astype(BF16).T

    def add_rows(j, p, o):
        rows = TC // NP
        tok = pl.ds(pl.multiple_of(j * TC + p * rows, rows), rows)
        xnew = xres[tok, :] + o
        xres[tok, :] = xnew
        xio[tok, :] = xnew.astype(BF16)

    def attention(last):
        for n in range(LEAD):
            step(None, None, n, n)

        def steps(i):
            for u in range(BODY):
                n = i * BODY + u
                step(n, u % RING, n + LEAD, (u + LEAD) % RING)
        _loop((NSTEP - LEAD) // BODY, steps)

        lhs[...] = gather_o(0)

        def tail(j):
            o = gather_o(j + 1)
            rows = TC // NP

            def between(c):
                if c % (NC // NP) == 0:
                    p = c // (NC // NP)
                    a = _pace(j < 0, lhs[p * rows:(p + 1) * rows, :], o, p, 2)
                    add_rows(j, p, jnp.dot(a, bwo[...], preferred_element_type=F32))
            step(NSTEP - LEAD + j, j, None, None, between)
            lhs[...] = o
            pl.when(last)(out_copy(j).start)
        _loop(LEAD, tail)

        def rest(i):
            j = i + LEAD
            o = gather_o(nxt(j))
            for p, piece in enumerate(_paced_dot(i < 0, lhs[...], bwo, o)):
                add_rows(j, p, piece)
            lhs[...] = o
            pl.when(last)(out_copy(j).start)
        _loop(NQ - LEAD, rest)

        @pl.when(jnp.logical_not(last))
        def _():
            xn1[...] = norm(0)

    in_copy(0).start()
    cp_wk.start()
    in_copy(0).wait()
    for i in range(1, NQ):
        in_copy(i).start()
    xres[_chunk(0), :] = xio[_chunk(0), :].astype(F32)
    xn1[...] = norm(0)

    def rep(r):
        first = r == 0
        zsum[...] = jnp.zeros(zsum.shape, F32)

        @pl.when(first)
        def _():
            cp_wk.wait()
            cp_wv.start()
            cp_wq.start()

        def k_pass(i):
            @pl.when(jnp.logical_and(first, i + 1 < NQ))
            def _():
                in_copy(nxt(i)).wait()
                xres[_chunk(nxt(i)), :] = xio[_chunk(nxt(i)), :].astype(F32)
            lin_k(i)
        _loop(NQ, k_pass)

        @pl.when(first)
        def _():
            cp_wv.wait()
            cp_wq.wait()
            cp_ao.start()
            cp_bw.start()
            cp_bo.start()
            transpose_qv(awqkv, awqvt)

        kvt[...] = jnp.zeros(kvt.shape, F32)
        _loop(NQ, lin_qv)

        @pl.when(first)
        def _():
            cp_ao.wait()
            cp_bw.wait()
            cp_bo.wait()
            transpose_qv(bwqkv, bwqvt)

        fold_kv()
        lhs[...] = scaled_q(0)
        _loop(NQ - 1, lambda i: lin_out(i, i < 0))
        lin_out(NQ - 1, r < 0, True)
        _loop(NQ, mha_qkv)
        attention(r == 1)

    _loop(2, rep)
    for i in range(NQ):
        out_copy(i).wait()


@jax.jit
def pallas_interleave_layers__linear_attn_block__mha_block__prompt_kernel(
    A_x: jax.Array,
    A_wqkv: jax.Array,
    A_wo: jax.Array,
    B_x: jax.Array,
    B_wqkv: jax.Array,
    B_wo: jax.Array,
):
    del B_x
    any_spec = pl.BlockSpec(memory_space=pl.ANY)
    out = pl.pallas_call(
        _kernel,
        out_shape=jax.ShapeDtypeStruct((S, D), BF16),
        in_specs=[any_spec] * 5,
        out_specs=any_spec,
        scratch_shapes=[
            pltpu.VMEM((S, D), BF16),
            pltpu.VMEM((D, 3 * D), BF16),
            pltpu.VMEM((D, D), BF16),
            pltpu.VMEM((D, 3 * D), BF16),
            pltpu.VMEM((D, D), BF16),
            pltpu.VMEM((2 * D, D), BF16),
            pltpu.VMEM((2 * D, D), BF16),
            pltpu.VMEM((S, D), F32),
            pltpu.VMEM((S, D), BF16),
            pltpu.VMEM((TC, D), BF16),
            pltpu.VMEM((S, D), BF16),
            pltpu.VMEM((D, S), F32),
            pltpu.VMEM((NSLAB, S, 128), BF16),
            pltpu.VMEM((H, 24, S), F32),
            pltpu.VMEM((H, 24, S), F32),
            pltpu.VMEM((TC, D), BF16),
            pltpu.VMEM((NSLAB, 64, S), jnp.int32),
            pltpu.VMEM((RING, S, TC), F32),
            pltpu.VMEM((RING, 8, TC), F32),
            pltpu.VMEM((D, D), F32),
            pltpu.VMEM((8, D), F32),
            pltpu.VMEM((D, D), BF16),
            pltpu.VMEM((H, D), BF16),
            pltpu.SemaphoreType.DMA((10,)),
        ],
        compiler_params=pltpu.CompilerParams(vmem_limit_bytes=110 * 1024 * 1024),
        name="interleave_layers",
    )(A_x.reshape(S, D), A_wqkv, A_wo, B_wqkv, B_wo)
    return out.reshape(1, S, D)
```

```python
import jax
import jax.numpy as jnp
from jax import lax
import jax.experimental.pallas as pl
import jax.experimental.pallas.tpu as pltpu

S, D, H, DH = 2048, 640, 32, 20
TC = 512
NQ = S // TC
BK = 128
NC = S // BK
LEAD = 2
RING = LEAD + 1
BODY = 9
NSTEP = H * NQ
assert (NSTEP - LEAD) % BODY == 0 and BODY % RING == 0
NSLAB = 6
NTILE = D // 128
NP = 8
F32, BF16 = jnp.float32, jnp.bfloat16
LOG2E = 1.4426950408889634
NN = (((1,), (0,)), ((), ()))
NT = (((1,), (1,)), ((), ()))
TN = (((0,), (0,)), ((), ()))


def _bands():
    out = []
    for j in range(NTILE):
        h0 = (128 * j) // DH
        h1 = -(-(128 * (j + 1)) // DH)
        out.append(((h0 * DH) // 16 * 16, min(D, -(-(h1 * DH) // 16) * 16)))
    return out


def _layernorm(x):
    m = jnp.mean(x, axis=-1, keepdims=True)
    xc = x - m
    v = jnp.mean(xc * xc, axis=-1, keepdims=True)
    return xc * lax.rsqrt(v + 1e-5)


def _phi(t):
    return jnp.where(t > 0, t + 1.0, jnp.exp(t)) + 1e-6


def _rnd(t):
    return t.astype(BF16).astype(F32)


def _recip(l):
    r = pltpu.reciprocal(l, approx=True)
    return r * (2.0 - l * r)


def _head_of(i):
    return (i * 3277) >> 16


def _pace(never, a, side, p, first):
    rows = a.shape[0]
    n = side.shape[0] // rows
    for t in range(n):
        if first + t * (NP - first) // n == p:
            a = jnp.where(never, side[t * rows:(t + 1) * rows], a)
    return a


def _paced_dot(never, lhs, rhs, side, dims=NN, first=2):
    rows = lhs.shape[0] // NP
    return [lax.dot_general(_pace(never, lhs[p * rows:(p + 1) * rows], side, p, first), rhs[...],
                            dims, preferred_element_type=F32) for p in range(NP)]


def _rows(i, n):
    if isinstance(i, int):
        return pl.ds(i * n, n)
    return pl.ds(pl.multiple_of(i * n, n), n)


def _chunk(i):
    return _rows(i, TC)


def _loop(n, body):
    def wrapped(i, c):
        body(i)
        return c
    lax.fori_loop(0, n, wrapped, 0)


def _kernel(x_hbm, awqkv_hbm, awo_hbm, bwqkv_hbm, bwo_hbm, out_hbm,
            xio, awqkv, awo, bwqkv, bwo, awt, bwt, xres, xn, xn1,
            ks, vt, ot, lhs, qs, sbuf, mbuf, kx, zsum, mmat, sems):
    def col_copy(part, sem):
        cols = slice(part * D, (part + 1) * D)
        return pltpu.make_async_copy(awqkv_hbm.at[:, cols], awqkv.at[:, cols], sems.at[sem])

    def in_copy(i):
        return pltpu.make_async_copy(x_hbm.at[_chunk(i), :], xio.at[_chunk(i), :], sems.at[i])

    def out_copy(i):
        half = _rows(i, TC // 2)
        return pltpu.make_async_copy(xio.at[half, :], out_hbm.at[half, :], sems.at[i])

    cp_wq, cp_wk, cp_wv = col_copy(0, 4), col_copy(1, 5), col_copy(2, 6)
    cp_ao = pltpu.make_async_copy(awo_hbm, awo, sems.at[7])
    cp_bw = pltpu.make_async_copy(bwqkv_hbm, bwqkv, sems.at[8])
    cp_bo = pltpu.make_async_copy(bwo_hbm, bwo, sems.at[9])

    def transposed(w, part):
        return jnp.concatenate(
            [w[:, c:c + 128].T for c in range(part * D, (part + 1) * D, 128)], axis=0)

    def norm(i):
        return _layernorm(xres[_chunk(i), :]).astype(BF16)

    def nxt(i):
        return jnp.minimum(i + 1, NQ - 1)

    def project_t(never, wt, x, side):
        return jnp.concatenate(
            [lax.dot_general(wt[:D - TC, :], x, NT, preferred_element_type=F32)]
            + _paced_dot(never, wt[D - TC:D, :], x, side, NT, 0), axis=0)

    def lin_k(i, first):
        tok = _chunk(nxt(i))
        xin = jnp.where(first, xio[tok, :].astype(F32), xres[tok, :])
        xres[tok, :] = xin
        y = _layernorm(xin).astype(BF16)
        x = xn1[...]
        xn[_chunk(i), :] = x
        pk = _phi(project_t(i < 0, awt, x, y))
        zsum[...] = jnp.where(i > 0, zsum[...], 0.0) + sum(
            pk[:, 128 * t:128 * (t + 1)] for t in range(TC // 128))
        kx[...] = jnp.where(i > 0, kx[...], 0.0) + jnp.dot(
            pk.astype(BF16), x, preferred_element_type=F32)
        xn1[...] = y

    def head_sums():
        zsum[...] = jnp.broadcast_to(jnp.sum(zsum[...], axis=1, keepdims=True), (D, 128))
        kvb = []
        for j, (r0, r1) in enumerate(_bands()):
            kvt = lax.dot_general(awt[2 * D + r0:2 * D + r1, :],
                                  kx[128 * j:128 * (j + 1), :].astype(BF16),
                                  NT, preferred_element_type=F32)
            re = _head_of(lax.broadcasted_iota(jnp.int32, (r1 - r0, 128), 0) + r0)
            cd = _head_of(lax.broadcasted_iota(jnp.int32, (r1 - r0, 128), 1) + 128 * j)
            kvb.append(jnp.where(re == cd, kvt, 0.0).astype(BF16))
        return kvb

    def fold_wo(kvb):
        for j, (r0, r1) in enumerate(_bands()):
            mmat[128 * j:128 * (j + 1), :] = lax.dot_general(
                kvb[j], awo[r0:r1, :], TN, preferred_element_type=F32).astype(BF16)

    def phi_q(i):
        return _phi(lax.dot_general(awt[D:2 * D, :], xn[_chunk(i), :], NT,
                                    preferred_element_type=F32))

    def scaled_q(pq):
        row = lax.broadcasted_iota(jnp.int32, (8, TC), 0)
        t = pq * jnp.concatenate([zsum[...]] * (TC // 128), axis=1)
        den = []
        for b in range(0, D, 2 * DH):
            mid = t[b + 16:b + 24]
            den += [t[b:b + 8] + t[b + 8:b + 16] + jnp.where(row < 4, mid, 0.0),
                    jnp.where(row < 4, 0.0, mid) + t[b + 24:b + 32] + t[b + 32:b + 40]]
        den = jnp.concatenate([jnp.sum(x, axis=0, keepdims=True) for x in den], axis=0) + 1e-6
        rden = 1.0 / den
        parts = []
        for j in range(H // 2):
            r0 = jnp.broadcast_to(rden[2 * j:2 * j + 1], (8, TC))
            r1 = jnp.broadcast_to(rden[2 * j + 1:2 * j + 2], (8, TC))
            parts += [r0, r0, jnp.where(row < 4, r0, r1), r1, r1]
        return (pq * jnp.concatenate(parts, axis=0)).astype(BF16).T

    def lin_out(i):
        side = scaled_q(phi_q(i + 1))
        xres[_chunk(i), :] += jnp.concatenate(_paced_dot(i < 0, lhs[...], mmat, side), axis=0)
        lhs[...] = side

    def lin_out_last(never):
        y = norm(0)
        wt = jnp.concatenate([transposed(bwqkv, 0), transposed(bwqkv, 2)], axis=0)
        bwt[...] = wt
        a, rows = lhs[...], TC // NP
        a = jnp.concatenate(
            [_pace(never, a[p * rows:(p + 1) * rows], wt, p, 1) for p in range(NP)], axis=0)
        xres[_chunk(NQ - 1), :] += jnp.concatenate(_paced_dot(never, a, mmat, y), axis=0)
        xn1[...] = y

    def mha_qkv(i):
        tok = _chunk(i)
        y = norm(nxt(i))
        x = xn1[...]
        k = jnp.dot(x, bwqkv[:, D:2 * D], preferred_element_type=F32)
        lane = lax.broadcasted_iota(jnp.int32, (TC, 128), 1)
        ks[0, tok, :] = k[:, :128].astype(BF16)
        ks[NSLAB - 1, tok, :] = k[:, D - 128:].astype(BF16)
        for s in range(1, NSLAB - 1):
            mix = jnp.where(lane >= 128 - 8 * s,
                            k[:, 128 * (s - 1):128 * s], k[:, 128 * s:128 * (s + 1)])
            ks[s, tok, :] = pltpu.roll(mix, 8 * s, 1).astype(BF16)
        v = _rnd(lax.dot_general(bwt[D:, :], x, NT, preferred_element_type=F32))
        row = lax.broadcasted_iota(jnp.int32, (8, TC), 0)
        for j in range(H // 2):
            b = 40 * j
            vt[2 * j, 0:16, tok] = v[b:b + 16]
            vt[2 * j, 16:24, tok] = jnp.where(row < 4, v[b + 16:b + 24], 1.0)
            w = [pltpu.roll(v[b + 16 + 8 * t:b + 24 + 8 * t], 4, 0) for t in range(3)] + [1.0]
            for t in range(3):
                vt[2 * j + 1, 8 * t:8 * t + 8, tok] = jnp.where(row < 4, w[t], w[t + 1])
        q = project_t(i < 0, bwt, x, y) * (LOG2E * DH ** -0.5)
        for s in range(NSLAB):
            st = min(120 * s, D - 128)
            qs[s, :, tok] = pltpu.bitcast(q[st:st + 128].astype(BF16), jnp.int32)
        xn1[...] = y

    def step(n_pv, b_pv, n_qk, b_qk, between=None):
        do_pv, do_qk = n_pv is not None, n_qk is not None
        if do_qk:
            h = n_qk >> 2
            sl = (h * 43) >> 8
            off = h * DH - jnp.minimum(sl * 120, D - 128)
            r = lax.broadcasted_iota(jnp.int32, (64, TC), 0) * 2
            q = jnp.where((r >= off) & (r < off + DH), qs[sl, :, _chunk(n_qk & 3)], 0)
            q = pltpu.bitcast(q, BF16)
            m_new = jnp.full((8, TC), -jnp.inf, F32)
        if do_pv:
            hv = n_pv >> 2
            m = jnp.max(mbuf[b_pv], axis=0, keepdims=True)
            acc = jnp.zeros((24, TC), F32)
        for c in range(NC):
            ck = slice(c * BK, (c + 1) * BK)
            if between is not None:
                between(c)
            if do_qk:
                s = jnp.dot(ks[sl, ck, :], q, preferred_element_type=F32)
                sbuf[b_qk, ck, :] = s
                m_new = jnp.maximum(m_new, jnp.max(s.reshape(BK // 8, 8, TC), axis=0))
            if do_pv:
                p = jnp.exp2(sbuf[b_pv, ck, :] - m).astype(BF16)
                acc = acc + jnp.dot(vt[hv, :, ck], p, preferred_element_type=F32)
        if do_qk:
            mbuf[b_qk] = m_new
        if do_pv:
            ot[hv, :, _chunk(n_pv & 3)] = acc

    def gather_o(j):
        tok = _chunk(j)
        row = lax.broadcasted_iota(jnp.int32, (8, TC), 0)
        parts = []
        for p in range(H // 2):
            e, o = ot[2 * p, :, tok], ot[2 * p + 1, :, tok]
            e, o = e * _recip(e[DH:DH + 1]), o * _recip(o[DH:DH + 1])
            w = [e[16:24]] + [pltpu.roll(o[8 * t:8 * t + 8], 4, 0) for t in range(3)]
            parts += [e[0:16]] + [jnp.where(row < 4, w[t], w[t + 1]) for t in range(3)]
        return jnp.concatenate(parts, axis=0).astype(BF16).T

    def add_rows(j, p, o, last):
        tok = _rows(j * NP + p, TC // NP)
        xnew = xres[tok, :] + o
        xres[tok, :] = xnew
        xio[tok, :] = xnew.astype(BF16)
        if (p + 1) % (NP // 2) == 0:
            pl.when(last)(out_copy(2 * j + p // (NP // 2)).start)

    def attention(last, never):
        for n in range(LEAD):
            step(None, None, n, n)

        def steps(i):
            for u in range(BODY):
                n = i * BODY + u
                step(n, u % RING, n + LEAD, (u + LEAD) % RING)
        _loop((NSTEP - LEAD) // BODY, steps)

        lhs[...] = gather_o(0)

        def tail(j):
            o = gather_o(j + 1)
            rows = TC // NP

            def between(c):
                if c % (NC // NP) == 0:
                    p = c // (NC // NP)
                    a = _pace(j < 0, lhs[p * rows:(p + 1) * rows, :], o, p, 2)
                    add_rows(j, p, jnp.dot(a, bwo[...], preferred_element_type=F32), last)
            step(NSTEP - LEAD + j, j, None, None, between)
            lhs[...] = o
        _loop(LEAD, tail)

        for j in range(LEAD, NQ):
            side = gather_o(j + 1) if j + 1 < NQ else norm(0)
            for p, piece in enumerate(_paced_dot(never, lhs[...], bwo, side)):
                add_rows(j, p, piece, last)
            (lhs if j + 1 < NQ else xn1)[...] = side

    in_copy(0).start()
    cp_wk.start()
    in_copy(1).start()

    def clear(i):
        n = (S - TC) // 8
        xres[pl.ds(pl.multiple_of(TC + i * n, 8), n), :] = jnp.zeros((n, D), F32)
        kx[_rows(i, D // 8), :] = jnp.zeros((D // 8, D), F32)
        zsum[_rows(i, D // 8), :] = jnp.zeros((D // 8, 128), F32)
    _loop(8, clear)

    in_copy(0).wait()
    cp_wk.wait()
    xres[_chunk(0), :] = xio[_chunk(0), :].astype(F32)
    xn1[...] = norm(0)
    awt[:D, :] = transposed(awqkv, 1)

    def rep(r):
        first = r == 0

        def k_pass(i):
            @pl.when(jnp.logical_and(first, i + 1 < NQ))
            def _():
                in_copy(nxt(i)).wait()

            @pl.when(jnp.logical_and(first, i == 0))
            def _():
                for c in range(2, NQ):
                    in_copy(c).start()
                cp_wv.start()
                cp_wq.start()

            @pl.when(jnp.logical_and(first, i == 1))
            def _():
                cp_ao.start()
                cp_bw.start()
                cp_bo.start()
            lin_k(i, first)
        _loop(NQ, k_pass)

        @pl.when(first)
        def _():
            cp_wv.wait()
            cp_wq.wait()
            cp_ao.wait()
            cp_bw.wait()
            cp_bo.wait()
            awt[D:2 * D, :] = transposed(awqkv, 0)
            awt[2 * D:, :] = transposed(awqkv, 2)

        pq = phi_q(0)
        kvb = head_sums()
        lhs[...] = scaled_q(pq)
        fold_wo(kvb)
        _loop(NQ - 1, lin_out)
        lin_out_last(r < 0)
        _loop(NQ, mha_qkv)
        attention(r == 1, r < 0)

    _loop(2, rep)
    for i in range(2 * NQ):
        out_copy(i).wait()


@jax.jit
def pallas_interleave_layers__linear_attn_block__mha_block__prompt_kernel(
    A_x: jax.Array,
    A_wqkv: jax.Array,
    A_wo: jax.Array,
    B_x: jax.Array,
    B_wqkv: jax.Array,
    B_wo: jax.Array,
):
    del B_x
    any_spec = pl.BlockSpec(memory_space=pl.ANY)
    out = pl.pallas_call(
        _kernel,
        out_shape=jax.ShapeDtypeStruct((S, D), BF16),
        in_specs=[any_spec] * 5,
        out_specs=any_spec,
        scratch_shapes=[
            pltpu.VMEM((S, D), BF16),
            pltpu.VMEM((D, 3 * D), BF16),
            pltpu.VMEM((D, D), BF16),
            pltpu.VMEM((D, 3 * D), BF16),
            pltpu.VMEM((D, D), BF16),
            pltpu.VMEM((3 * D, D), BF16),
            pltpu.VMEM((2 * D, D), BF16),
            pltpu.VMEM((S, D), F32),
            pltpu.VMEM((S, D), BF16),
            pltpu.VMEM((TC, D), BF16),
            pltpu.VMEM((NSLAB, S, 128), BF16),
            pltpu.VMEM((H, 24, S), F32),
            pltpu.VMEM((H, 24, S), F32),
            pltpu.VMEM((TC, D), BF16),
            pltpu.VMEM((NSLAB, 64, S), jnp.int32),
            pltpu.VMEM((RING, S, TC), F32),
            pltpu.VMEM((RING, 8, TC), F32),
            pltpu.VMEM((D, D), F32),
            pltpu.VMEM((D, 128), F32),
            pltpu.VMEM((D, D), BF16),
            pltpu.SemaphoreType.DMA((10,)),
        ],
        compiler_params=pltpu.CompilerParams(vmem_limit_bytes=110 * 1024 * 1024),
        name="interleave_layers",
    )(A_x.reshape(S, D), A_wqkv, A_wo, B_wqkv, B_wo)
    return out.reshape(1, S, D)
```
